```python
import os as _os
_os.environ.setdefault("JAX_PLATFORMS", "cpu")
import jax
import jax.numpy as jnp

def _softmax(x, axis=-1):
    return jax.nn.softmax(x, axis=axis)
def _gelu(x):
    return jax.nn.gelu(x, approximate=True)
def _silu(x):
    return jax.nn.silu(x)
def _sigmoid(x):
    return jax.nn.sigmoid(x)
def _layernorm(x, axis=-1, eps=1e-5):
    m = jnp.mean(x, axis=axis, keepdims=True)
    v = jnp.var(x, axis=axis, keepdims=True)
    return (x - m) / jnp.sqrt(v + eps)
def _scatter_add(tgt, idx, src, axis=0):
    return tgt.at[idx].add(src)
def _segment_sum(src, seg, n):
    return jax.ops.segment_sum(src, seg, n)
class _Rng:
    def __init__(self, key):
        self._k = key
    def _next(self):
        self._k, sub = jax.random.split(self._k)
        return sub
    def normal(self, shape):
        return jax.random.normal(self._next(), shape, dtype=jnp.bfloat16)
    def randint(self, lo, hi, shape):
        return jax.random.randint(self._next(), shape, lo, hi, dtype=jnp.int32)
    def uniform(self, shape, lo=0.0, hi=1.0):
        return jax.random.uniform(self._next(), shape, jnp.bfloat16, lo, hi)
    def permutation(self, n):
        return jax.random.permutation(self._next(), n)


kernel_name = 'gated_mix__mha_block__mha_block__prompt'

def setup_inputs():
    _rng = _Rng(jax.random.key(int.from_bytes(__import__("os").urandom(4), "little")))
    _w = (lambda a: (lambda t: t.astype(jnp.bfloat16) if jnp.issubdtype(t.dtype, jnp.floating) else t)(jnp.asarray(a)))
    def _A_setup():
        B, S, D, H = 1, 2048, 448, 16
        return {
            "x": _w((lambda *s: _rng.normal(s) * 0.05)(B, S, D)),
            "wqkv": _w((lambda *s: _rng.normal(s) * 0.4)(D, 3 * D)),
            "wo": _w((lambda *s: _rng.normal(s) * 0.05)(D, D)),
        }
    _A_in = _A_setup()

    def _B_setup():
        B, S, D, H = 1, 2048, 448, 16
        return {
            "x": _w((lambda *s: _rng.normal(s) * 0.05)(B, S, D)),
            "wqkv": _w((lambda *s: _rng.normal(s) * 0.4)(D, 3 * D)),
            "wo": _w((lambda *s: _rng.normal(s) * 0.05)(D, D)),
        }
    _B_in = _B_setup()

    return {
        "A_x": _A_in["x"],
        "A_wqkv": _A_in["wqkv"],
        "A_wo": _A_in["wo"],
        "B_x": _B_in["x"],
        "B_wqkv": _B_in["wqkv"],
        "B_wo": _B_in["wo"],
        "gate_w": _w((lambda *s: _rng.normal(s) * 0.05)(448) * 16.0),
    }

def reference(A_x, A_wqkv, A_wo, B_x, B_wqkv, B_wo, gate_w):
    def _A_ref(x, wqkv, wo):
        B, S, D = x.shape
        H = 16
        Dh = D // H
        qkv = (lambda x, *d: x.transpose(*d))((x @ wqkv).reshape(B, S, 3, H, Dh), 2, 0, 3, 1, 4)
        q, k, v = qkv[0], qkv[1], qkv[2]
        scores = jnp.einsum("bhqd,bhkd->bhqk", q, k) * (Dh ** -0.5)
        p = _softmax(scores, axis=-1)
        o = jnp.einsum("bhqk,bhkd->bhqd", p, v)
        return (lambda x, *d: x.transpose(*d))(o, 0, 2, 1, 3).reshape(B, S, D) @ wo

    def _B_ref(x, wqkv, wo):
        B, S, D = x.shape
        H = 16
        Dh = D // H
        qkv = (lambda x, *d: x.transpose(*d))((x @ wqkv).reshape(B, S, 3, H, Dh), 2, 0, 3, 1, 4)
        q, k, v = qkv[0], qkv[1], qkv[2]
        scores = jnp.einsum("bhqd,bhkd->bhqk", q, k) * (Dh ** -0.5)
        p = _softmax(scores, axis=-1)
        o = jnp.einsum("bhqk,bhkd->bhqd", p, v)
        return (lambda x, *d: x.transpose(*d))(o, 0, 2, 1, 3).reshape(B, S, D) @ wo

    x = A_x
    g = _sigmoid((x * gate_w).sum(-1, keepdims=True))
    a = _A_ref(x, A_wqkv, A_wo)
    b = _B_ref(x, B_wqkv, B_wo)
    return g * a + (1 - g) * b
```

```python
import functools, math
import jax, jax.numpy as jnp
from jax import lax
from jax.experimental import pallas as pl
from jax.experimental.pallas import tpu as pltpu

S, D, H, DH, DP = 2048, 448, 16, 28, 32
NH = 2 * H
NG = NH // 4
LOG2E = 1.4426950408889634
F32, BF16 = jnp.float32, jnp.bfloat16

def make(CK=128, SUB=512, PQ=512, scopes=False):
    NC = S // CK
    NP = S // PQ
    scale = (DH ** -0.5) * LOG2E
    import contextlib
    scope = (lambda n: jax.named_scope(n)) if scopes else (lambda n: contextlib.nullcontext())

    def kernel(xT_hbm, wa_hbm, wb_hbm, woa_hbm, wob_hbm, gw_ref, o_hbm,
               k_s, vT_s, qm_s, oT_s, sA, sB, mA, mB, g_s,
               xT_ref, wa_ref, wb_ref, woa_ref, wob_ref, o_ref, wk_s, wo_s, sem_in, sem_out):
        cps = [pltpu.make_async_copy(src, dst, sem_in.at[n]) for n, (src, dst) in enumerate(
            ((wa_hbm, wa_ref), (wb_hbm, wb_ref), (xT_hbm, xT_ref), (woa_hbm, woa_ref), (wob_hbm, wob_ref)))]
        for cp in cps:
            cp.start()
        with scope("wkprep"):
            r = lax.broadcasted_iota(jnp.int32, (512, 512), 0) + 384 - D
            c = lax.broadcasted_iota(jnp.int32, (512, 512), 1)
            E = jnp.where((r == (c // DP) * DH + (c % DP)) & ((c % DP) < DH), 1.0, 0.0).astype(BF16)
            for b, w_ref in enumerate((wa_ref, wb_ref)):
                cps[b].wait()
                wk_s[:, 512 * b:512 * (b + 1)] = jnp.dot(w_ref[:, 384:896], E, preferred_element_type=F32).astype(BF16)
            cps[2].wait()

        tail_v = jnp.concatenate([jnp.ones((1, PQ), F32), jnp.zeros((3, PQ), F32)], axis=0)
        gw = jnp.broadcast_to(gw_ref[...], (8, D))
        def proj(qi, carry):
            cols = pl.ds(pl.multiple_of(qi * PQ, PQ), PQ)
            xq = xT_ref[:, cols]
            k = jnp.dot(xq.T, wk_s[...], preferred_element_type=F32)
            for j in range(NG):
                k_s[j, cols, :] = k[:, 128 * j:128 * (j + 1)].astype(BF16)
            for b, w_ref in enumerate((wa_ref, wb_ref)):
                wq = w_ref[:, 0:D]
                wv = w_ref[:, 2 * D:3 * D]
                vT = lax.dot_general(wv, xq, (((0,), (0,)), ((), ())), preferred_element_type=F32)
                qT = lax.dot_general(wq, xq, (((0,), (0,)), ((), ())), preferred_element_type=F32) * scale
                for h in range(H):
                    vh = jnp.concatenate([vT[DH * h:DH * (h + 1)], tail_v], axis=0)
                    vT_s[b * H + h, :, cols] = vh.astype(BF16)
                    a = h % 4
                    parts = []
                    if a > 0:
                        parts.append(jnp.zeros((DP * a, PQ), F32))
                    parts.append(qT[DH * h:DH * (h + 1)])
                    parts.append(jnp.zeros((128 - DP * a - DH, PQ), F32))
                    qm_s[b * H + h, :, cols] = jnp.concatenate(parts, axis=0).astype(BF16)
            g = jax.nn.sigmoid(jnp.dot(gw, xq, preferred_element_type=F32))
            g_s[0, :, cols] = g
            g_s[1, :, cols] = 1.0 - g
            return carry
        with scope("proj"):
            lax.fori_loop(0, NP, proj, 0)

        def stage(tq, so, mo, tf, si, mi):
            if tq is not None:
                j = tq // 4
            for u in range(S // SUB):
                cols = pl.ds(u * SUB, SUB)
                if tq is not None:
                    qm = qm_s[tq, :, cols]
                mpart = None
                acc = None
                if tf is not None:
                    m_in = mi[0:1, cols]
                for c in range(NC):
                    rows = pl.ds(c * CK, CK)
                    if tq is not None:
                        sT = jnp.dot(k_s[j, rows, :], qm, preferred_element_type=F32)
                        so[rows, cols] = sT
                        mc = jnp.max(sT.reshape(CK // 8, 8, SUB), axis=0)
                        mpart = mc if mpart is None else jnp.maximum(mpart, mc)
                    if tf is not None:
                        pT = jnp.exp2(si[rows, cols] - m_in).astype(BF16)
                        o = jnp.dot(vT_s[tf, :, rows], pT, preferred_element_type=F32)
                        acc = o if acc is None else acc + o
                if tf is not None:
                    gate = g_s[tf // H, 0:1, cols]
                    l = acc[DH:DH + 1, :]
                    oT_s[tf, :, cols] = (acc * (gate / l)).astype(BF16)
                if tq is not None:
                    mo[:, cols] = jnp.broadcast_to(jnp.max(mpart, axis=0, keepdims=True), (8, SUB))

        with scope("stage0"):
            stage(0, sA, mA, None, None, None)
        def body(t, c):
            @pl.when(t % 2 == 0)
            def _():
                stage(t + 1, sB, mB, t, sA, mA)
            @pl.when(t % 2 == 1)
            def _():
                stage(t + 1, sA, mA, t, sB, mB)
            return c
        with scope("mainloop"):
            lax.fori_loop(0, NH - 1, body, 0)
        with scope("laststage"):
            stage(None, None, None, NH - 1, sB, mB)

        with scope("outproj"):
            cps[3].wait()
            cps[4].wait()
            z4 = jnp.zeros((DP - DH, D), BF16)
            parts = []
            for wo_ref in (woa_ref, wob_ref):
                for h in range(H):
                    parts.append(wo_ref[DH * h:DH * (h + 1), :])
                    parts.append(z4)
            wo_s[...] = jnp.concatenate(parts, axis=0).T
            def oproj(qi, carry):
                cols = pl.ds(pl.multiple_of(qi * PQ, PQ), PQ)
                oT = oT_s[:, :, cols].reshape(NH * DP, PQ)
                outT = jnp.dot(wo_s[...], oT, preferred_element_type=F32)
                o_ref[:, cols] = outT.astype(o_ref.dtype)
                pltpu.make_async_copy(o_ref.at[:, cols], o_hbm.at[:, cols], sem_out.at[qi]).start()
                return carry
            lax.fori_loop(0, NP, oproj, 0)
            for qi in range(NP):
                cols = slice(qi * PQ, (qi + 1) * PQ)
                pltpu.make_async_copy(o_ref.at[:, cols], o_hbm.at[:, cols], sem_out.at[qi]).wait()

    def fn(A_x, A_wqkv, A_wo, B_x, B_wqkv, B_wo, gate_w):
        xT = jnp.swapaxes(A_x, 1, 2).reshape(D, S)
        out = pl.pallas_call(
            kernel,
            out_shape=jax.ShapeDtypeStruct((D, S), BF16),
            in_specs=[pl.BlockSpec(memory_space=pl.ANY)] * 5 + [pl.BlockSpec(memory_space=pltpu.VMEM)],
            out_specs=pl.BlockSpec(memory_space=pl.ANY),
            scratch_shapes=[
                pltpu.VMEM((NG, S, 128), BF16),
                pltpu.VMEM((NH, DP, S), BF16),
                pltpu.VMEM((NH, 128, S), BF16),
                pltpu.VMEM((NH, DP, S), BF16),
                pltpu.VMEM((S, S), F32),
                pltpu.VMEM((S, S), F32),
                pltpu.VMEM((8, S), F32),
                pltpu.VMEM((8, S), F32),
                pltpu.VMEM((2, 8, S), F32),
                pltpu.VMEM((D, S), BF16),
                pltpu.VMEM((D, 3 * D), BF16),
                pltpu.VMEM((D, 3 * D), BF16),
                pltpu.VMEM((D, D), BF16),
                pltpu.VMEM((D, D), BF16),
                pltpu.VMEM((D, S), BF16),
                pltpu.VMEM((D, NH * DP), BF16),
                pltpu.VMEM((D, NH * DP), BF16),
                pltpu.SemaphoreType.DMA((5,)),
                pltpu.SemaphoreType.DMA((NP,)),
            ],
            compiler_params=pltpu.CompilerParams(
                vmem_limit_bytes=110 * 1024 * 1024),
        )(xT, A_wqkv, B_wqkv, A_wo, B_wo, gate_w.reshape(1, D))
        return jnp.swapaxes(out.reshape(1, D, S), 1, 2)
    return fn


_fn = make()


@jax.jit
def pallas_gated_mix__mha_block__mha_block__prompt_kernel(
    A_x: jax.Array,
    A_wqkv: jax.Array,
    A_wo: jax.Array,
    B_x: jax.Array,
    B_wqkv: jax.Array,
    B_wo: jax.Array,
    gate_w: jax.Array,
):
    return _fn(A_x, A_wqkv, A_wo, B_x, B_wqkv, B_wo, gate_w)
```

```python
import jax
import jax.numpy as jnp
from jax import lax
import jax.experimental.pallas as pl
import jax.experimental.pallas.tpu as pltpu

S, D, H, DH, DP = 2048, 448, 16, 28, 32
NH = 2 * H
NG = NH // 4
LOG2E = 1.4426950408889634
F32, BF16 = jnp.float32, jnp.bfloat16

CK = 128
SUB = 512
PQ = 512
NC = S // CK
NP = S // PQ
QSCALE = (DH ** -0.5) * LOG2E


def _kernel(xT_hbm, wa_hbm, wb_hbm, woa_hbm, wob_hbm, gw_ref, o_hbm,
            k_s, vT_s, qm_s, oT_s, sA, sB, mA, mB, g_s,
            xT_ref, wa_ref, wb_ref, woa_ref, wob_ref, o_ref, wo_s, wT_s,
            sem_in, sem_x, sem_out):
    def xcopy(qi):
        cols = pl.ds(pl.multiple_of(qi * PQ, PQ), PQ)
        return pltpu.make_async_copy(xT_hbm.at[:, cols], xT_ref.at[:, cols], sem_x.at[qi])

    cps = [pltpu.make_async_copy(src, dst, sem_in.at[n]) for n, (src, dst) in enumerate(
        ((wa_hbm, wa_ref), (wb_hbm, wb_ref), (woa_hbm, woa_ref), (wob_hbm, wob_ref)))]
    cps[0].start()
    for qi in range(NP):
        xcopy(qi).start()
    for cp in cps[1:]:
        cp.start()

    tail_v = jnp.concatenate([jnp.ones((1, PQ), F32), jnp.zeros((DP - DH - 1, PQ), F32)], axis=0)
    gw = jnp.broadcast_to(gw_ref[...], (8, D))

    for b, w_ref in enumerate((wa_ref, wb_ref)):
        cps[b].wait()
        wT_s[...] = w_ref[...].T

        def proj(qi, carry, b=b):
            cols = pl.ds(pl.multiple_of(qi * PQ, PQ), PQ)
            if b == 0:
                xcopy(qi).wait()
            xq = xT_ref[:, cols]
            qkvT = jnp.dot(wT_s[...], xq, preferred_element_type=F32)
            qT = qkvT[0:D] * QSCALE
            vT = qkvT[2 * D:3 * D]
            z4 = jnp.zeros((DP - DH, PQ), F32)
            for j in range(4):
                parts = []
                for h in range(4 * j, 4 * j + 4):
                    parts += [qkvT[D + DH * h:D + DH * (h + 1)], z4]
                k_s[4 * b + j, cols, :] = jnp.concatenate(parts, axis=0).T.astype(BF16)
            for h in range(H):
                vh = jnp.concatenate([vT[DH * h:DH * (h + 1)], tail_v], axis=0)
                vT_s[b * H + h, :, cols] = vh.astype(BF16)
                a = h % 4
                parts = []
                if a > 0:
                    parts.append(jnp.zeros((DP * a, PQ), F32))
                parts.append(qT[DH * h:DH * (h + 1)])
                parts.append(jnp.zeros((128 - DP * a - DH, PQ), F32))
                qm_s[b * H + h, :, cols] = jnp.concatenate(parts, axis=0).astype(BF16)
            if b == 0:
                g = jax.nn.sigmoid(jnp.dot(gw, xq, preferred_element_type=F32))
                g_s[0, :, cols] = g
                g_s[1, :, cols] = 1.0 - g
            return carry

        lax.fori_loop(0, NP, proj, 0)

    def stage(tq, so, mo, tf, si, mi):
        if tq is not None:
            j = tq // 4
        for u in range(S // SUB):
            cols = pl.ds(u * SUB, SUB)
            if tq is not None:
                qm = qm_s[tq, :, cols]
            mpart = None
            acc = None
            if tf is not None:
                m_in = mi[0:1, cols]
            for c in range(NC):
                rows = pl.ds(c * CK, CK)
                if tq is not None:
                    sT = jnp.dot(k_s[j, rows, :], qm, preferred_element_type=F32)
                    so[rows, cols] = sT
                    mc = jnp.max(sT.reshape(CK // 8, 8, SUB), axis=0)
                    mpart = mc if mpart is None else jnp.maximum(mpart, mc)
                if tf is not None:
                    pT = jnp.exp2(si[rows, cols] - m_in).astype(BF16)
                    o = jnp.dot(vT_s[tf, :, rows], pT, preferred_element_type=F32)
                    acc = o if acc is None else acc + o
            if tf is not None:
                gate = g_s[tf // H, 0:1, cols]
                denom = acc[DH:DH + 1, :]
                oT_s[tf, :, cols] = (acc * (gate / denom)).astype(BF16)
            if tq is not None:
                mo[:, cols] = jnp.broadcast_to(jnp.max(mpart, axis=0, keepdims=True), (8, SUB))

    cps[2].wait()
    cps[3].wait()
    zrow = jnp.zeros((DP - DH, D), BF16)
    parts = []
    for wo_ref in (woa_ref, wob_ref):
        for h in range(H):
            parts.append(wo_ref[DH * h:DH * (h + 1), :])
            parts.append(zrow)
    wo_s[...] = jnp.concatenate(parts, axis=0).T

    stage(0, sA, mA, None, None, None)

    def body(i, carry):
        t = 2 * i
        stage(t + 1, sB, mB, t, sA, mA)
        stage(t + 2, sA, mA, t + 1, sB, mB)
        return carry

    lax.fori_loop(0, NH // 2 - 1, body, 0)
    stage(NH - 1, sB, mB, NH - 2, sA, mA)
    stage(None, None, None, NH - 1, sB, mB)

    def oproj(qi, carry):
        cols = pl.ds(pl.multiple_of(qi * PQ, PQ), PQ)
        oT = oT_s[:, :, cols].reshape(NH * DP, PQ)
        outT = jnp.dot(wo_s[...], oT, preferred_element_type=F32)
        o_ref[:, cols] = outT.astype(o_ref.dtype)
        pltpu.make_async_copy(o_ref.at[:, cols], o_hbm.at[:, cols], sem_out.at[qi]).start()
        return carry

    lax.fori_loop(0, NP, oproj, 0)
    for qi in range(NP):
        cols = slice(qi * PQ, (qi + 1) * PQ)
        pltpu.make_async_copy(o_ref.at[:, cols], o_hbm.at[:, cols], sem_out.at[qi]).wait()


@jax.jit
def pallas_gated_mix__mha_block__mha_block__prompt_kernel(
    A_x: jax.Array,
    A_wqkv: jax.Array,
    A_wo: jax.Array,
    B_x: jax.Array,
    B_wqkv: jax.Array,
    B_wo: jax.Array,
    gate_w: jax.Array,
):
    xT = jnp.swapaxes(A_x, 1, 2).reshape(D, S)
    outT = pl.pallas_call(
        _kernel,
        out_shape=jax.ShapeDtypeStruct((D, S), BF16),
        in_specs=[pl.BlockSpec(memory_space=pl.ANY)] * 5 + [pl.BlockSpec(memory_space=pltpu.VMEM)],
        out_specs=pl.BlockSpec(memory_space=pl.ANY),
        scratch_shapes=[
            pltpu.VMEM((NG, S, 128), BF16),
            pltpu.VMEM((NH, DP, S), BF16),
            pltpu.VMEM((NH, 128, S), BF16),
            pltpu.VMEM((NH, DP, S), BF16),
            pltpu.VMEM((S, S), F32),
            pltpu.VMEM((S, S), F32),
            pltpu.VMEM((8, S), F32),
            pltpu.VMEM((8, S), F32),
            pltpu.VMEM((2, 8, S), F32),
            pltpu.VMEM((D, S), BF16),
            pltpu.VMEM((D, 3 * D), BF16),
            pltpu.VMEM((D, 3 * D), BF16),
            pltpu.VMEM((D, D), BF16),
            pltpu.VMEM((D, D), BF16),
            pltpu.VMEM((D, S), BF16),
            pltpu.VMEM((D, NH * DP), BF16),
            pltpu.VMEM((3 * D, D), BF16),
            pltpu.SemaphoreType.DMA((4,)),
            pltpu.SemaphoreType.DMA((NP,)),
            pltpu.SemaphoreType.DMA((NP,)),
        ],
        compiler_params=pltpu.CompilerParams(vmem_limit_bytes=110 * 1024 * 1024),
    )(xT, A_wqkv, B_wqkv, A_wo, B_wo, gate_w.reshape(1, D))
    return jnp.swapaxes(outT.reshape(1, D, S), 1, 2)
```

```python
import jax
import jax.numpy as jnp
from jax import lax
import jax.experimental.pallas as pl
import jax.experimental.pallas.tpu as pltpu

S, D, H, DH, DP = 2048, 448, 16, 28, 32
NH = 2 * H
NG = NH // 4
LOG2E = 1.4426950408889634
F32, BF16 = jnp.float32, jnp.bfloat16

CK = 128
SUB = 512
PQ = 512
NC = S // CK
NP = S // PQ
QSCALE = (DH ** -0.5) * LOG2E


def _kernel(xT_hbm, wa_hbm, wb_hbm, woa_hbm, wob_hbm, gw_ref, o_hbm,
            k_s, vT_s, qm_s, oT_s, sA, sB, mA, mB, g_s,
            xT_ref, wa_ref, wb_ref, woa_ref, wob_ref, o_ref, wo_s, wT_s,
            sem_in, sem_x, sem_out):
    def xcopy(qi):
        cols = pl.ds(pl.multiple_of(qi * PQ, PQ), PQ)
        return pltpu.make_async_copy(xT_hbm.at[:, cols], xT_ref.at[:, cols], sem_x.at[qi])

    cps = [pltpu.make_async_copy(src, dst, sem_in.at[n]) for n, (src, dst) in enumerate(
        ((wa_hbm, wa_ref), (wb_hbm, wb_ref), (woa_hbm, woa_ref), (wob_hbm, wob_ref)))]
    cps[0].start()
    for qi in range(NP):
        xcopy(qi).start()
    for cp in cps[1:]:
        cp.start()

    for hh in range(NH):
        a = hh % 4
        if a > 0:
            qm_s[hh, 0:DP * a, :] = jnp.zeros((DP * a, S), BF16)
        if a < 3:
            qm_s[hh, DP * (a + 1):128, :] = jnp.zeros((128 - DP * (a + 1), S), BF16)

    tail_v = jnp.concatenate([jnp.ones((1, PQ), F32), jnp.zeros((DP - DH - 1, PQ), F32)], axis=0)
    gw = jnp.broadcast_to(gw_ref[...], (8, D))

    for b, w_ref in enumerate((wa_ref, wb_ref)):
        cps[b].wait()
        wT_s[...] = w_ref[...].T

        def proj(qi, carry, b=b):
            cols = pl.ds(pl.multiple_of(qi * PQ, PQ), PQ)
            if b == 0:
                xcopy(qi).wait()
            xq = xT_ref[:, cols]
            qkvT = jnp.dot(wT_s[...], xq, preferred_element_type=F32)
            qT = qkvT[0:D] * QSCALE
            vT = qkvT[2 * D:3 * D]
            z4 = jnp.zeros((DP - DH, PQ), F32)
            for j in range(4):
                parts = []
                for h in range(4 * j, 4 * j + 4):
                    parts += [qkvT[D + DH * h:D + DH * (h + 1)], z4]
                k_s[4 * b + j, cols, :] = jnp.concatenate(parts, axis=0).T.astype(BF16)
            for h in range(H):
                vh = jnp.concatenate([vT[DH * h:DH * (h + 1)], tail_v], axis=0)
                vT_s[b * H + h, :, cols] = vh.astype(BF16)
                a = h % 4
                qm_s[b * H + h, DP * a:DP * (a + 1), cols] = jnp.concatenate(
                    [qT[DH * h:DH * (h + 1)], z4], axis=0).astype(BF16)
            if b == 0:
                g = jax.nn.sigmoid(jnp.dot(gw, xq, preferred_element_type=F32))
                g_s[0, :, cols] = g
                g_s[1, :, cols] = 1.0 - g
            return carry

        lax.fori_loop(0, NP, proj, 0)

    def stage(tq, so, mo, tf, si, mi):
        if tq is not None:
            j = tq // 4
        for u in range(S // SUB):
            cols = pl.ds(u * SUB, SUB)
            if tq is not None:
                qm = qm_s[tq, :, cols]
            mpart = None
            acc = None
            if tf is not None:
                m_in = mi[0:1, cols]
            for c in range(NC):
                rows = pl.ds(c * CK, CK)
                if tq is not None:
                    sT = jnp.dot(k_s[j, rows, :], qm, preferred_element_type=F32)
                    so[rows, cols] = sT
                    mc = jnp.max(sT.reshape(CK // 8, 8, SUB), axis=0)
                    mpart = mc if mpart is None else jnp.maximum(mpart, mc)
                if tf is not None:
                    pT = jnp.exp2(si[rows, cols] - m_in).astype(BF16)
                    o = jnp.dot(vT_s[tf, :, rows], pT, preferred_element_type=F32)
                    acc = o if acc is None else acc + o
            if tf is not None:
                gate = g_s[tf // H, 0:1, cols]
                denom = acc[DH:DH + 1, :]
                oT_s[tf, :, cols] = (acc * (gate / denom)).astype(BF16)
            if tq is not None:
                mo[:, cols] = jnp.broadcast_to(jnp.max(mpart, axis=0, keepdims=True), (8, SUB))

    cps[2].wait()
    cps[3].wait()
    zrow = jnp.zeros((DP - DH, D), BF16)
    parts = []
    for wo_ref in (woa_ref, wob_ref):
        for h in range(H):
            parts.append(wo_ref[DH * h:DH * (h + 1), :])
            parts.append(zrow)
    wo_s[...] = jnp.concatenate(parts, axis=0).T

    stage(0, sA, mA, None, None, None)

    def body(i, carry):
        t = 2 * i
        stage(t + 1, sB, mB, t, sA, mA)
        stage(t + 2, sA, mA, t + 1, sB, mB)
        return carry

    lax.fori_loop(0, NH // 2 - 1, body, 0)
    stage(NH - 1, sB, mB, NH - 2, sA, mA)
    stage(None, None, None, NH - 1, sB, mB)

    def oproj(qi, carry):
        cols = pl.ds(pl.multiple_of(qi * PQ, PQ), PQ)
        oT = oT_s[:, :, cols].reshape(NH * DP, PQ)
        outT = jnp.dot(wo_s[...], oT, preferred_element_type=F32)
        o_ref[:, cols] = outT.astype(o_ref.dtype)
        pltpu.make_async_copy(o_ref.at[:, cols], o_hbm.at[:, cols], sem_out.at[qi]).start()
        return carry

    lax.fori_loop(0, NP, oproj, 0)
    for qi in range(NP):
        cols = slice(qi * PQ, (qi + 1) * PQ)
        pltpu.make_async_copy(o_ref.at[:, cols], o_hbm.at[:, cols], sem_out.at[qi]).wait()


@jax.jit
def pallas_gated_mix__mha_block__mha_block__prompt_kernel(
    A_x: jax.Array,
    A_wqkv: jax.Array,
    A_wo: jax.Array,
    B_x: jax.Array,
    B_wqkv: jax.Array,
    B_wo: jax.Array,
    gate_w: jax.Array,
):
    xT = jnp.swapaxes(A_x, 1, 2).reshape(D, S)
    outT = pl.pallas_call(
        _kernel,
        out_shape=jax.ShapeDtypeStruct((D, S), BF16),
        in_specs=[pl.BlockSpec(memory_space=pl.ANY)] * 5 + [pl.BlockSpec(memory_space=pltpu.VMEM)],
        out_specs=pl.BlockSpec(memory_space=pl.ANY),
        scratch_shapes=[
            pltpu.VMEM((NG, S, 128), BF16),
            pltpu.VMEM((NH, DP, S), BF16),
            pltpu.VMEM((NH, 128, S), BF16),
            pltpu.VMEM((NH, DP, S), BF16),
            pltpu.VMEM((S, S), F32),
            pltpu.VMEM((S, S), F32),
            pltpu.VMEM((8, S), F32),
            pltpu.VMEM((8, S), F32),
            pltpu.VMEM((2, 8, S), F32),
            pltpu.VMEM((D, S), BF16),
            pltpu.VMEM((D, 3 * D), BF16),
            pltpu.VMEM((D, 3 * D), BF16),
            pltpu.VMEM((D, D), BF16),
            pltpu.VMEM((D, D), BF16),
            pltpu.VMEM((D, S), BF16),
            pltpu.VMEM((D, NH * DP), BF16),
            pltpu.VMEM((3 * D, D), BF16),
            pltpu.SemaphoreType.DMA((4,)),
            pltpu.SemaphoreType.DMA((NP,)),
            pltpu.SemaphoreType.DMA((NP,)),
        ],
        compiler_params=pltpu.CompilerParams(vmem_limit_bytes=110 * 1024 * 1024),
    )(xT, A_wqkv, B_wqkv, A_wo, B_wo, gate_w.reshape(1, D))
    return jnp.swapaxes(outT.reshape(1, D, S), 1, 2)
```
